```python
import jax
import jax.numpy as jnp

def _softmax(x, axis=-1):
    return jax.nn.softmax(x, axis=axis)
def _gelu(x):
    return jax.nn.gelu(x, approximate=True)
def _silu(x):
    return jax.nn.silu(x)
def _sigmoid(x):
    return jax.nn.sigmoid(x)
def _layernorm(x, axis=-1, eps=1e-5):
    m = jnp.mean(x, axis=axis, keepdims=True)
    v = jnp.var(x, axis=axis, keepdims=True)
    return (x - m) / jnp.sqrt(v + eps)
def _scatter_add(tgt, idx, src, axis=0):
    return tgt.at[idx].add(src)
def _segment_sum(src, seg, n):
    return jax.ops.segment_sum(src, seg, n)
class _Rng:
    def __init__(self, key):
        self._k = key
    def _next(self):
        self._k, sub = jax.random.split(self._k)
        return sub
    def normal(self, shape):
        return jax.random.normal(self._next(), shape, dtype=jnp.bfloat16)
    def randint(self, lo, hi, shape):
        return jax.random.randint(self._next(), shape, lo, hi, dtype=jnp.int32)
    def uniform(self, shape, lo=0.0, hi=1.0):
        return jax.random.uniform(self._next(), shape, jnp.bfloat16, lo, hi)
    def permutation(self, n):
        return jax.random.permutation(self._next(), n)


kernel_name = 'sequential_preLN__spectral_gfnet__swiglu_ffn__prompt'

def _fwd_setup_inputs():
    _rng = _Rng(jax.random.key(int.from_bytes(__import__("os").urandom(4), "little")))
    _w = (lambda a: (lambda t: t.astype(jnp.bfloat16) if jnp.issubdtype(t.dtype, jnp.floating) else t)(jnp.asarray(a)))
    def _A_setup():
        B, S, D = 1, 2048, 576
        Df = D // 2 + 1
        return {
            "x": _w((lambda *s: _rng.normal(s) * 0.05)(B, S, D)),
            "w_r": _w((lambda *s: _rng.normal(s) * 0.05)(S, Df) * 0.02),
            "w_i": _w((lambda *s: _rng.normal(s) * 0.05)(S, Df) * 0.02),
        }
    _A_in = _A_setup()

    def _B_setup():
        B, S, D, F = 1, 2048, 576, 4608
        return {
            "x": _w((lambda *s: _rng.normal(s) * 0.05)(B, S, D)),
            "w_gate": _w((lambda *s: _rng.normal(s) * 0.05)(D, F)),
            "w_up": _w((lambda *s: _rng.normal(s) * 0.05)(D, F)),
            "w_down": _w((lambda *s: _rng.normal(s) * 0.05)(F, D)),
        }
    _B_in = _B_setup()

    return {
        "A_x": _A_in["x"],
        "A_w_r": _A_in["w_r"],
        "A_w_i": _A_in["w_i"],
        "B_x": _B_in["x"],
        "B_w_gate": _B_in["w_gate"],
        "B_w_up": _B_in["w_up"],
        "B_w_down": _B_in["w_down"],
    }

def _fwd_reference(A_x, A_w_r, A_w_i, B_x, B_w_gate, B_w_up, B_w_down):
    def _A_ref(x, w_r, w_i):
        B, S, D = x.shape
        X = (lambda x, axes=(-2,-1): jnp.fft.rfft2(x.astype(jnp.float32), axes=axes))(x, axes=(-2, -1))
        W = w_r + 1j * w_i
        X = X * W
        y = (lambda x, s, axes=(-2,-1): jnp.fft.irfft2(x, s=s, axes=axes).astype(jnp.bfloat16))(X, (S, D), axes=(-2, -1))
        return y

    def _B_ref(x, w_gate, w_up, w_down):
        g = _silu(x @ w_gate)
        u = x @ w_up
        return (g * u) @ w_down

    x = A_x
    h = x + _A_ref(_layernorm(x, axis=-1), A_w_r, A_w_i)
    h2 = h + _B_ref(_layernorm(h, axis=-1), B_w_gate, B_w_up, B_w_down)
    return h2


def setup_inputs():
    _inp = _fwd_setup_inputs()
    _gk = jax.random.fold_in(jax.random.key(int.from_bytes(__import__("os").urandom(4), "little")), 2**31 - 1)
    _shapes = [[1, 2048, 576]]
    _dtypes = ['bfloat16']
    _gks = jax.random.split(_gk, len(_shapes))
    _gs = [jax.random.normal(k, s, dtype=jnp.dtype(d)) * 0.05 for k, s, d in zip(_gks, _shapes, _dtypes)]
    _inp["grad_out"] = _gs[0]
    return _inp

def reference(A_x, A_w_r, A_w_i, B_w_gate, B_w_up, B_w_down, B_x, grad_out):
    _const = dict(B_x=B_x)
    def _f(*_d):
        return _fwd_reference(**{'A_x': _d[0], 'A_w_r': _d[1], 'A_w_i': _d[2], 'B_w_gate': _d[3], 'B_w_up': _d[4], 'B_w_down': _d[5], **_const})
    _out, _vjp = jax.vjp(_f, A_x, A_w_r, A_w_i, B_w_gate, B_w_up, B_w_down)
    _grads = _vjp(grad_out)
    _out0 = jnp.asarray(_out)
    return (_out0, *[jnp.asarray(_g) for _g in _grads])
```

```python
import numpy as np
import jax
import jax.numpy as jnp
import jax.experimental.pallas as pl
import jax.experimental.pallas.tpu as pltpu
import ml_dtypes

S, D, F = 2048, 576, 4608
SH = S // 2
DF = D // 2 + 1
FP = 304
TF = 512
FH = TF // 2
NF = F // TF
SC = 256
SUB = SC // 2
NC = SH // SC
EPS = 1e-5
BF = jnp.bfloat16
F32 = jnp.float32

_CLS = [(0, 0, 64), (3, 64, 48), (1, 112, 48), (5, 160, 48), (2, 208, 48), (4, 256, 48)]
_GRP = [(0, 64, 0, 96), (64, 48, 96, 96), (112, 96, 192, 192), (208, 96, 384, 192)]


def _consts():
    rows = np.full((FP,), -1)
    for r, o, n in _CLS:
        f = r + 6 * np.arange(n)
        rows[o:o + n] = np.where(f < DF, f, -1)
    d2 = np.arange(96)[None, :]
    cm = np.zeros((8, 192, 256), np.float64)
    h3 = np.sqrt(3.0) / 2
    for gi, (o, n, _, k) in enumerate(_GRP):
        f = rows[o:o + n][:, None]
        e = np.where(f >= 0, np.exp(-2j * np.pi * ((f * d2) % D) / D), 0.0)
        if k == 192:
            sgn = np.where((f % 6) < 3, -1.0, 1.0)
            e = np.concatenate([e, e * 1j * h3 * sgn], axis=1)
        m = np.concatenate([e.real, e.imag], axis=0)
        cm[gi, :2 * n, :k] = m
        cm[4 + gi, :k, :2 * n] = m.T
    g = np.zeros((16, 256, 256), np.float64)
    lane = np.arange(128)
    s2 = np.arange(128)[:, None]
    for k1 in range(16):
        t = (lane - k1) % 16
        j = ((lane - t - k1) % 128) // 16
        k = (128 * t + 16 * j + k1)[None, :]
        a = 2.0 * np.pi * ((s2 * k) % S) / S
        gr, gi = np.cos(a), -np.sin(a)
        g[k1, :128, :128] = gr
        g[k1, :128, 128:] = gi
        g[k1, 128:, :128] = -gi
        g[k1, 128:, 128:] = gr
    c = lambda z: z.astype(np.float32).astype(ml_dtypes.bfloat16)
    return c(cm), c(g)


_CM, _G = _consts()
_NT = (((1,), (1,)), ((), ()))


def _dot(a, b):
    return jnp.dot(a, b, preferred_element_type=F32)


def _dot_nt(a, b):
    return jax.lax.dot_general(a, b, _NT, preferred_element_type=F32)


def _lc(a11, a12, a21, a22):
    return [a11 + a22, a21 + a22, a11, a22, a11 + a12, a21 - a11, a12 - a22]


def _rc(b11, b12, b21, b22):
    return [b11 + b22, b11, b12 - b22, b21 - b11, b22, b11 + b12, b21 + b22]


def _mc(c11, c12, c21, c22):
    return [c11 + c22, c21 - c22, c12 + c22, c11 + c21, c12 - c11, c22, c11]


def _post(m):
    return m[0] + m[3] - m[4] + m[6], m[2] + m[4], m[1] + m[3], m[0] - m[1] + m[2] + m[5]


def _post_l(m):
    return m[0] + m[2] + m[4] - m[5], m[4] + m[6], m[1] + m[5], m[0] + m[1] + m[3] - m[6]


def _post_r(m):
    return m[0] + m[1] - m[3] + m[5], m[2] + m[5], m[3] + m[6], m[0] - m[2] + m[4] + m[6]


_REM1 = (0, 1, 2, 5)
_REM2 = (0, 1, 3, 6)


def _radix4(x, sign):
    (ar, ai), (br, bi), (cr, ci), (dr, di) = x
    t0r, t0i, t1r, t1i = ar + cr, ai + ci, ar - cr, ai - ci
    t2r, t2i, t3r, t3i = br + dr, bi + di, br - dr, bi - di
    p = (t1r + t3i, t1i - t3r)
    m = (t1r - t3i, t1i + t3r)
    y1, y3 = (p, m) if sign < 0 else (m, p)
    return [(t0r + t2r, t0i + t2i), y1, (t0r - t2r, t0i - t2i), y3]


def _twiddle(z, e, sign):
    r, i = z
    if e == 0:
        return z
    if e == 4:
        return (i, -r) if sign < 0 else (-i, r)
    c = float(np.cos(2 * np.pi * e / 16))
    s = float(sign * np.sin(2 * np.pi * e / 16))
    if e in (2, 6):
        return ((r - i) * c, (r + i) * c) if c * s > 0 else ((r + i) * c, (i - r) * c)
    return (r * c - i * s, r * s + i * c)


def _fft16(x, sign):
    a = [_radix4([x[b], x[4 + b], x[8 + b], x[12 + b]], sign) for b in range(4)]
    out = [None] * 16
    for c in range(4):
        y = _radix4([_twiddle(a[b][c], b * c, sign) for b in range(4)], sign)
        for d in range(4):
            out[c + 4 * d] = y[d]
    return out


def _radix6(n):
    n = [n[96 * j:96 * (j + 1)] for j in range(6)]
    e = [n[j] + n[j + 3] for j in range(3)]
    o = [n[j] - n[j + 3] for j in range(3)]
    es, od = e[1] + e[2], o[1] - o[2]
    return [e[0] + es, o[0] - od, o[0] + 0.5 * od, o[1] + o[2], e[0] - 0.5 * es, e[1] - e[2]]


def _radix6_adj(t):
    t0, t3, p1, q1, p2, q2 = t
    es, od = t0 - 0.5 * p2, 0.5 * p1 - t3
    e = [t0 + p2, es + q2, es - q2]
    o = [t3 + p1, q1 + od, q1 - od]
    return jnp.concatenate([e[j] + o[j] for j in range(3)]
                           + [e[j] - o[j] for j in range(3)], axis=0)


def _barrel(v, cls):
    w = [v[(-m) % 16] for m in range(16)]
    for b in range(4):
        m = (cls & (1 << b)) != 0
        w = [jnp.where(m, w[(i - (1 << b)) % 16], w[i]) for i in range(16)]
    return w


def _ln(x):
    m = jnp.mean(x, axis=0, keepdims=True)
    xc = x - m
    v = jnp.mean(xc * xc, axis=0, keepdims=True)
    r = jax.lax.rsqrt(v + EPS)
    return xc * r, r


def _ln_bwd(dn, n, r):
    return r * (dn - jnp.mean(dn, axis=0, keepdims=True)
                - n * jnp.mean(dn * n, axis=0, keepdims=True))


def _split(a):
    return (jnp.concatenate([a[:256], a[512:544]], axis=0),
            jnp.concatenate([a[256:512], a[544:]], axis=0))


def _join(a, b):
    return jnp.concatenate([a[:256], b[:256], a[256:], b[256:]], axis=0)


def _loop(n, body):
    def step(i, c):
        body(i)
        return c
    jax.lax.fori_loop(0, n, step, 0)


def _ds(start, n):
    return pl.ds(pl.multiple_of(start, n), n)


def _kernel(x_hbm, go_hbm, wr_hbm, wi_hbm, cm_hbm, g_hbm, wg_hbm, wu_hbm, wd_hbm,
            out_hbm, dx_hbm, dwr_hbm, dwi_hbm, dwg_hbm, dwu_hbm, dwd_hbm,
            xT, goT, w_io, cm, g, wp, wf, tb, z, zb, xs, h, obuf,
            lnT, mgT, ln, mg, rem, hacc, dacc, wacc, m, dm, rw, wst, gst,
            zs, sems, wsem, gsem):
    w_hbm = (wg_hbm, wu_hbm, wd_hbm)
    dw_hbm = (dwg_hbm, dwu_hbm, dwd_hbm)
    XC = 512

    def x_copy(c):
        return pltpu.make_async_copy(x_hbm.at[:, _ds(c * XC, XC)], xT.at[:, _ds(c * XC, XC)],
                                     sems.at[c])

    def dx_copy(c):
        return pltpu.make_async_copy(tb.at[:, _ds(c * XC, XC)], dx_hbm.at[:, _ds(c * XC, XC)],
                                     sems.at[c])

    cm_copy = pltpu.make_async_copy(cm_hbm, cm, sems.at[4])
    g_copy = pltpu.make_async_copy(g_hbm, g, sems.at[5])
    go_copy = pltpu.make_async_copy(go_hbm, goT, sems.at[6])
    wr_copy = pltpu.make_async_copy(wr_hbm, w_io.at[0], sems.at[7])
    wi_copy = pltpu.make_async_copy(wi_hbm, w_io.at[1], sems.at[8])
    out_copy = pltpu.make_async_copy(obuf, out_hbm, sems.at[6])
    dwr_copy = pltpu.make_async_copy(w_io.at[0], dwr_hbm, sems.at[7])
    dwi_copy = pltpu.make_async_copy(w_io.at[1], dwi_hbm, sems.at[8])

    def w_copies(j):
        return [pltpu.make_async_copy(w_hbm[i].at[:, _ds(j * TF, TF)], wst.at[(j % 2) * 3 + i],
                                      wsem.at[(j % 2) * 3 + i]) for i in range(3)]

    def dw_copies(j):
        return [pltpu.make_async_copy(gst.at[(j % 2) * 3 + i], dw_hbm[i].at[:, _ds(j * TF, TF)],
                                      gsem.at[(j % 2) * 3 + i]) for i in range(3)]

    def start(cs):
        for c in cs:
            c.start()

    def wait(cs):
        for c in cs:
            c.wait()

    def class_rows(i):
        f0 = 96 * i
        for r, o, _ in _CLS[1:]:
            f0 = jnp.where(i >= o // 16, r + 96 * (i - o // 16), f0)
        return pl.ds(f0, 16, stride=6)

    def wcomb_pieces(b, q):
        def pair(i, c, ra, rb, rd):
            lo, hi = slice(c, c + 128), slice(FH + c, FH + c + 128)
            w = [wst[b * 3 + i, r, cs].astype(F32) for r in (ra, rb) for cs in (lo, hi)]
            vs = _rc(*w) if i < 2 else _rc(w[0], w[2], w[1], w[3])
            for k in range(7):
                rw[b * 7 + k, rd, i * FH + c:i * FH + c + 128] = vs[k].astype(BF)

        def tail(i, c):
            rs = _ds(512 + q * 16, 16)
            top, bot = _ds(288 + q * 16, 16), _ds(352 + q * 16, 16)
            cs = slice(i * FH + c, i * FH + c + 128)
            u, v = wst[b * 3 + i, rs, c:c + 128], wst[b * 3 + i, rs, FH + c:FH + c + 128]
            rw[b * 7, top, cs] = u
            rw[b * 7 + 1, bot, cs] = u
            if i < 2:
                t = u.astype(F32) + v.astype(F32)
                rw[b * 7 + 2, top, cs] = v
                rw[b * 7 + 5, top, cs] = (-t).astype(BF)
                rw[b * 7 + 5, bot, cs] = t.astype(BF)
            else:
                t = (v.astype(F32) - u.astype(F32)).astype(BF)
                rw[b * 7 + 3, top, cs] = t
                rw[b * 7 + 3, bot, cs] = t
                rw[b * 7 + 6, top, cs] = v
        ps = []
        for i in range(3):
            for c in range(0, FH, 128):
                for r in range(0, 64, 16):
                    ra = _ds(q * 64 + r, 16)
                    ps.append(lambda i=i, c=c, ra=ra, r=r: pair(i, c, ra, _ds(256 + q * 64 + r, 16), ra))
                hq = (q % 2) * 16
                ps.append(lambda i=i, c=c: (pair(i, c, _ds(512 + hq, 16), _ds(544 + hq, 16),
                                                 _ds(256 + hq, 16)), tail(i, c)))
        return ps

    def wpost_pieces(b, q):
        def piece(i, c, rs, ra, rb):
            lo, hi = slice(c, c + 128), slice(FH + c, FH + c + 128)
            v = _post_r([wacc[b * 7 + k, rs, i * FH + c:i * FH + c + 128] for k in range(7)])
            if i == 2:
                v = (v[0], v[2], v[1], v[3])
            for t, (r, cs) in zip(v, ((ra, lo), (ra, hi), (rb, lo), (rb, hi))):
                gst[b * 3 + i, r, cs] = t.astype(BF)
        ps = []
        for i in range(3):
            for c in range(0, FH, 128):
                for r in range(0, 64, 16):
                    ra = _ds(q * 64 + r, 16)
                    ps.append(lambda i=i, c=c, ra=ra, r=r: piece(i, c, ra, ra, _ds(256 + q * 64 + r, 16)))
                hq = (q % 2) * 16
                ps.append(lambda i=i, c=c: piece(i, c, _ds(256 + hq, 16), _ds(512 + hq, 16),
                                                 _ds(544 + hq, 16)))
        return ps

    def put_radix6(n, cols):
        for j, t in enumerate(_radix6(n)):
            tb[96 * j:96 * (j + 1), cols] = t.astype(BF)

    def get_radix6_adj(cols):
        return _radix6_adj([z[96 * j:96 * (j + 1), cols] for j in range(6)])

    cls = jax.lax.broadcasted_iota(jnp.int32, (16, 128), 1) & 15

    def fwd_pre():
        start([x_copy(c) for c in range(S // XC)] + [cm_copy])
        zs[0] = 2
        wf[:, 288:] = jnp.zeros((16, 96, 128), F32)
        rw[:, 288:] = jnp.zeros((14, 128, 3 * FH), BF)

        def body(c):
            pl.when(c % 2 == 0)(lambda: x_copy(c // 2).wait())
            pl.when(c == 2)(lambda: start([wr_copy, wi_copy]))
            cols = _ds(c * 256, 256)
            put_radix6(_ln(xT[:, cols].astype(F32))[0], cols)
        _loop(8, body)
        g_copy.start()
        wait([wr_copy, wi_copy])

        def part(a):
            def cvt(c):
                for t in range(2):
                    wf[2 * c + t, :DF] = w_io[a, :, _ds(c * 256 + t * 128, 128)].astype(F32)
            _loop(8, cvt)

            def perm(i):
                rs = class_rows(i)
                v = [wf[t, rs] for t in range(16)]
                v = _barrel([v[0]] + [pltpu.roll(v[t], t, 1) for t in range(1, 16)], cls)
                for k in range(16):
                    wp[2 * k + a, _ds(i * 16, 16)] = v[k]
            _loop(FP // 16, perm)
        _loop(2, part)
        start([go_copy] + w_copies(0))
        wait([cm_copy, g_copy])

    def spectral(ph):
        def dfwd(c):
            cols = _ds(c * 1024, 1024)
            for gi, (o, n, t0, k) in enumerate(_GRP):
                v = _dot(cm[gi, :2 * n, :k], tb[t0:t0 + k, cols])
                z[o:o + n, cols] = v[:n]
                z[FP + o:FP + o + n, cols] = v[n:]
        _loop(2, dfwd)

        def load_z(i):
            return [(z[_ds(i * 16, 16), t * 128:(t + 1) * 128],
                     z[_ds(FP + i * 16, 16), t * 128:(t + 1) * 128]) for t in range(16)]

        def bfly(i):
            y = _fft16(load_z(i), -1)
            for k in range(16):
                zb[k, _ds(i * 16, 16), :128] = y[k][0].astype(BF)
                zb[k, _ds(i * 16, 16), 128:] = y[k][1].astype(BF)
        _loop(FP // 16, bfly)

        row = jax.lax.broadcasted_iota(jnp.int32, (FP, 128), 0)
        cf = jnp.where((row == 0) | (row == 48), 1.0 / (S * D), 2.0 / (S * D))
        sg = jnp.where(ph == 0, 1.0, -1.0)

        def mix(i):
            ys = []
            for kk in range(4):
                k = i * 4 + kk
                v = _dot(zb[k], g[k])
                vr, vi = v[:, :128], v[:, 128:]
                gr, gi = vr * cf, vi * cf
                xr, xi = xs[2 * k], xs[2 * k + 1]
                wr, wi = wp[2 * k], wp[2 * k + 1] * sg
                xs[2 * k] = jnp.where(ph == 0, vr, gr * xr + gi * xi)
                xs[2 * k + 1] = jnp.where(ph == 0, vi, gi * xr - gr * xi)
                ys.append(jnp.concatenate([(gr * wr - gi * wi).astype(BF),
                                           (gr * wi + gi * wr).astype(BF)], axis=1))
            for kk in range(4):
                k = i * 4 + kk
                v = _dot_nt(ys[kk], g[k])
                z[:FP, _ds(k * 128, 128)] = v[:, :128]
                z[FP:, _ds(k * 128, 128)] = v[:, 128:]
        _loop(4, mix)

        def ibfly(i):
            y = _fft16(load_z(i), 1)
            for t in range(16):
                cs = slice((t % 2) * 128, (t % 2 + 1) * 128)
                zb[t // 2, _ds(i * 16, 16), cs] = y[t][0].astype(BF)
                zb[8 + t // 2, _ds(i * 16, 16), cs] = y[t][1].astype(BF)
        _loop(FP // 16, ibfly)

        def dinv(c):
            cols = _ds(c * 1024, 1024)
            for gi, (o, n, t0, k) in enumerate(_GRP):
                rhs = jnp.concatenate(
                    [jnp.concatenate([zb[p + c * 4 + q, o:o + n] for q in range(4)], axis=1)
                     for p in (0, 8)], axis=0)
                z[t0:t0 + k, cols] = _dot(cm[4 + gi, :k, :2 * n], rhs)
        _loop(2, dinv)

    def fwd_post():
        start(w_copies(1))
        wait([go_copy] + w_copies(0))

        def body(c):
            ca, cb = _ds(c * 128, 128), _ds(SH + c * 128, 128)
            ns = []
            for cols in (ca, cb):
                hv = xT[:, cols].astype(F32) + get_radix6_adj(cols)
                h[:, cols] = hv
                ns.append(_ln(hv)[0])
            gs = [goT[:, cols].astype(F32) for cols in (ca, cb)]
            for i, (vals, comb, dst_t, dst) in enumerate(((ns, _lc, lnT, ln), (gs, _mc, mgT, mg))):
                for k, v in enumerate(comb(*_split(vals[0]), *_split(vals[1]))):
                    dst_t[k, :, ca] = v.astype(BF)
                    dst[k, ca] = v[:256].T.astype(BF)
                rem[i, ca] = jnp.concatenate([vals[0][512:], vals[1][512:]], axis=0).T.astype(BF)
        _loop(SH // 128, body)

        def comb(q):
            for p in wcomb_pieces(0, q):
                p()
        _loop(NC, comb)

    def ffn_iter(it):
        j, c = it // NC, it % NC
        b = j % 2
        s0 = c * SC

        @pl.when(c == 0)
        def _():
            pl.when(j + 1 < NF)(lambda: wait(w_copies(j + 1)))
            pl.when(j + 2 < NF)(lambda: start(w_copies(j + 2)))
            pl.when(j >= 2)(lambda: start(dw_copies(j - 2)))
            pl.when(j >= 3)(lambda: wait(dw_copies(j - 3)))

        parts = ((slice(0, TF), ln, lnT, dacc, _REM1), (slice(TF, 3 * FH), mg, mgT, hacc, _REM2))

        def p_dots(o):
            rs = _ds(s0 + o, SUB)

            def t(i, k):
                cs, lhs, _, _, has_rem = parts[i]
                if k in has_rem:
                    v = _dot(jnp.concatenate([lhs[k, rs], rem[i, rs]], axis=1),
                             jnp.concatenate([rw[b * 7 + k, :256, cs], rw[b * 7 + k, 288:, cs]], axis=0))
                else:
                    v = _dot(lhs[k, rs], rw[b * 7 + k, :256, cs])
                m[k, o:o + SUB, cs] = v
                return v
            return [lambda i=i, k=k: t(i, k) for i in range(2) for k in range(7)]

        def r_dots(o):
            rs = _ds(s0 + o, SUB)

            def t(i, k):
                cs, _, _, acc, _ = parts[i]
                v = (jnp.where(j == 0, 0.0, acc[k, :, rs])
                     + _dot_nt(rw[b * 7 + k, :288, cs], dm[k, o:o + SUB, cs]))
                acc[k, :, rs] = v
                return v
            return [lambda i=i, k=k: t(i, k) for i in range(2) for k in range(7)]

        def q_dots():
            def t(i, k):
                cs, _, lhs, _, _ = parts[i]
                v = (jnp.where(c == 0, 0.0, wacc[b * 7 + k, :, cs])
                     + _dot(lhs[k, :, _ds(s0, SC)], dm[k, :, cs]))
                wacc[b * 7 + k, :, cs] = v
                return v
            return [lambda i=i, k=k: t(i, k) for i in range(2) for k in range(7)]

        def ew_pieces(o):
            def piece(r, c0):
                rs = slice(r, r + 16)
                cs = [slice(i * FH + c0, i * FH + c0 + 128) for i in range(3)]
                a = _post([m[k, rs, cs[0]] for k in range(7)])
                u = _post([m[k, rs, cs[1]] for k in range(7)])
                dp = _post_l([m[k, rs, cs[2]] for k in range(7)])
                da, du, p = [], [], []
                for ai, ui, di in zip(a, u, dp):
                    s = 0.5 * jnp.tanh(0.5 * ai) + 0.5
                    gl = ai * s
                    p.append(gl * ui)
                    du.append(di * gl)
                    da.append((di * ui) * (s + gl * (1.0 - s)))
                for cc, vs in zip(cs, (_mc(*da), _mc(*du), _lc(*p))):
                    for k in range(7):
                        dm[k, rs, cc] = vs[k].astype(BF)
            return [lambda r=r, c0=c0: piece(r, c0)
                    for r in range(o, o + SUB, 16) for c0 in range(0, FH, 128)]

        def paced(dots, pieces, fence, frac=0.85):
            done, cum = 0, 0
            for t, w in zip(dots, [2] * 7 + [1] * 7):
                v = t()
                nr = v.shape[0] // 16
                while done < len(pieces) and done * 21 * frac < (cum + w) * len(pieces):
                    r = min(nr - 1, int((done * 21 * frac / len(pieces) - cum) / w * nr))
                    fence(v[r * 16:r * 16 + 16, :128])
                    pieces[done]()
                    done += 1
                cum += w

        zz = zs[0]

        def fence_m(v):
            m[zz + 5, :8, :128] = v[:8]

        def fence_wacc(v):
            wacc[zz + 12, :8, :128] = v[:8]

        def fence_wst(v):
            wst[zz + 4, :16, :128] = v.astype(BF)

        paced(p_dots(0), wpost_pieces(1 - b, c), fence_wacc)
        paced(p_dots(SUB), ew_pieces(0), fence_m)
        paced(r_dots(0), ew_pieces(SUB), fence_m)
        paced(r_dots(SUB), [], None)
        paced(q_dots(), wcomb_pieces(1 - b, c), fence_wst)

    def bwd_pre():
        start(dw_copies(NF - 2))

        def body(c):
            ca, cb = _ds(c * 128, 128), _ds(SH + c * 128, 128)
            f = _post([hacc[k, :, ca] for k in range(7)])
            dn = _post_l([dacc[k, :, ca] for k in range(7)])
            for i, cols in enumerate((ca, cb)):
                hv = h[:, cols]
                obuf[:, cols] = (hv + _join(f[2 * i], f[2 * i + 1])).astype(BF)
                n, r = _ln(hv)
                dh = goT[:, cols].astype(F32) + _ln_bwd(_join(dn[2 * i], dn[2 * i + 1]), n, r)
                h[:, cols] = dh
                put_radix6(dh, cols)
        _loop(SH // 128, body)
        out_copy.start()
        wait(dw_copies(NF - 3))

        def post(q):
            for p in wpost_pieces((NF - 1) % 2, q):
                p()
        _loop(NC, post)
        start(dw_copies(NF - 1))

    def bwd_post():
        def part(a):
            def unperm(i):
                v = _barrel([xs[2 * k + a, _ds(i * 16, 16)] for k in range(16)], cls)
                rs = class_rows(i)
                for t in range(16):
                    wf[t, rs] = pltpu.roll(v[t], 128 - t, 1) if t else v[t]
            _loop(FP // 16, unperm)

            def cvt(c):
                for t in range(2):
                    w_io[a, :, _ds(c * 256 + t * 128, 128)] = wf[2 * c + t, :DF].astype(BF)
            _loop(8, cvt)
        _loop(2, part)
        start([dwr_copy, dwi_copy])

        def body(c):
            cols = _ds(c * 256, 256)
            n, r = _ln(xT[:, cols].astype(F32))
            tb[:, cols] = (h[:, cols] + _ln_bwd(get_radix6_adj(cols), n, r)).astype(BF)
            pl.when(c % 2 == 1)(lambda: dx_copy(c // 2).start())
        _loop(8, body)
        wait([out_copy, dwr_copy, dwi_copy] + dw_copies(NF - 2) + dw_copies(NF - 1)
             + [dx_copy(c) for c in range(S // XC)])

    def phase(ph):
        pl.when(ph == 0)(fwd_pre)
        pl.when(ph == 1)(bwd_pre)
        spectral(ph)

        @pl.when(ph == 0)
        def _():
            fwd_post()
            _loop(NF * NC, ffn_iter)
        pl.when(ph == 1)(bwd_post)
    _loop(2, phase)


@jax.jit
def pallas_sequential_preLN__spectral_gfnet__swiglu_ffn__prompt_kernel(
    A_x, A_w_r, A_w_i, B_x, B_w_gate, B_w_up, B_w_down, grad_out,
):
    del B_x
    anyspec = pl.BlockSpec(memory_space=pl.ANY)
    sds = jax.ShapeDtypeStruct
    V = pltpu.VMEM
    outs = pl.pallas_call(
        _kernel,
        in_specs=[anyspec] * 9,
        out_specs=[anyspec] * 7,
        out_shape=[sds((D, S), BF), sds((D, S), BF), sds((DF, S), BF), sds((DF, S), BF),
                   sds((D, F), BF), sds((D, F), BF), sds((D, F), BF)],
        scratch_shapes=[
            V((D, S), BF),
            V((D, S), BF),
            V((2, DF, S), BF),
            V((8, 192, 256), BF),
            V((16, 256, 256), BF),
            V((32, FP, 128), F32),
            V((16, 384, 128), F32),
            V((D, S), BF),
            V((2 * FP, S), F32),
            V((16, FP, 256), BF),
            V((32, FP, 128), F32),
            V((D, S), F32),
            V((D, S), BF),
            V((7, 288, SH), BF),
            V((7, 288, SH), BF),
            V((7, SH, 256), BF),
            V((7, SH, 256), BF),
            V((2, SH, 128), BF),
            V((7, 288, SH), F32),
            V((7, 288, SH), F32),
            V((15, 288, 3 * FH), F32),
            V((8, SC, 3 * FH), F32),
            V((7, SC, 3 * FH), BF),
            V((14, 416, 3 * FH), BF),
            V((7, D, TF), BF),
            V((6, D, TF), BF),
            pltpu.SMEM((1,), jnp.int32),
            pltpu.SemaphoreType.DMA((9,)),
            pltpu.SemaphoreType.DMA((6,)),
            pltpu.SemaphoreType.DMA((6,)),
        ],
        compiler_params=pltpu.CompilerParams(vmem_limit_bytes=124 * 1024 * 1024),
        name="fused_gfnet_swiglu",
    )(A_x[0].T, grad_out[0].T, A_w_r.T, A_w_i.T, _CM, _G, B_w_gate, B_w_up, B_w_down.T)
    o, dx, dwr, dwi, dwg, dwu, dwd = outs
    return (o.T[None], dx.T[None], dwr.T, dwi.T, dwg, dwu, dwd.T)
```

```python
import numpy as np
import jax
import jax.numpy as jnp
import jax.experimental.pallas as pl
import jax.experimental.pallas.tpu as pltpu
import ml_dtypes

S, D, F = 2048, 576, 4608
SH = S // 2
DF = D // 2 + 1
FP = 304
TF = 512
FH = TF // 2
NF = F // TF
SC = 256
SUB = SC // 2
NC = SH // SC
XC = 512
EPS = 1e-5
BF = jnp.bfloat16
F32 = jnp.float32
U32 = jnp.uint32

_CLS = {0: (0, 64), 3: (64, 48), 1: (112, 48), 5: (160, 48), 2: (208, 48), 4: (256, 48)}
_GRP = [(0, 64, 0, 96), (64, 48, 96, 96), (112, 96, 192, 192), (208, 96, 384, 192)]
_PAIR = [(0, 56), (56, 48), (104, 48)]


def _words(z):
    z = z.astype(np.float32).astype(ml_dtypes.bfloat16).view(np.uint16).astype(np.uint32)
    return z[..., 0::2, :] | (z[..., 1::2, :] << 16)


def _consts():
    rows = np.full((FP,), -1)
    for r, (o, n) in _CLS.items():
        f = r + 6 * np.arange(n)
        rows[o:o + n] = np.where(f < DF, f, -1)
    d2 = np.arange(96)[None, :]
    cm = np.zeros((2, 4, 192, 256), np.float64)
    h3 = np.sqrt(3.0) / 2
    for gi, (o, n, _, k) in enumerate(_GRP):
        f = rows[o:o + n][:, None]
        e = np.where(f >= 0, np.exp(-2j * np.pi * ((f * d2) % D) / D), 0.0)
        if k == 192:
            sgn = np.where((f % 6) < 3, -1.0, 1.0)
            e = np.concatenate([e, e * 1j * h3 * sgn], axis=1)
        m = np.concatenate([e.real, e.imag], axis=0)
        cm[0, gi, :2 * n, :k] = m
        order = np.arange(2 * n).reshape(2, -1, 8).transpose(1, 0, 2).reshape(-1)
        cm[1, gi, :k, :2 * n] = m.T[:, order]
    g = np.zeros((16, 256, 256), np.float64)
    lane = np.arange(128)
    s2 = np.arange(128)[:, None]
    for k1 in range(16):
        t = (lane - k1) % 16
        j = ((lane - t - k1) % 128) // 16
        k = (128 * t + 16 * j + k1)[None, :]
        a = 2.0 * np.pi * ((s2 * k) % S) / S
        gr, gi = np.cos(a), -np.sin(a)
        g[k1, :128, :128] = gr
        g[k1, :128, 128:] = gi
        g[k1, 128:, :128] = -gi
        g[k1, 128:, 128:] = gr
    return _words(cm), _words(g)


_CM, _G = _consts()
_NT = (((1,), (1,)), ((), ()))


def _dot(a, b):
    return jnp.dot(a, b, preferred_element_type=F32)


def _dot_nt(a, b):
    return jax.lax.dot_general(a, b, _NT, preferred_element_type=F32)


def _bf(w):
    return pltpu.bitcast(w, BF)


def _wd(v):
    return pltpu.bitcast(v.astype(BF), U32)


def _half(w, i):
    return pltpu.bitcast(w & jnp.uint32(0xFFFF0000) if i else w << 16, F32)


def _both(a, b):
    bits = lambda v: pltpu.bitcast(v.astype(BF).astype(F32), U32)
    return (bits(a) >> 16) | bits(b)


def _stack(a, b):
    return _wd(jnp.concatenate([a, b], axis=0))


def _lc(a11, a12, a21, a22):
    return [a11 + a22, a21 + a22, a11, a22, a11 + a12, a21 - a11, a12 - a22]


def _rc(b11, b12, b21, b22):
    return [b11 + b22, b11, b12 - b22, b21 - b11, b22, b11 + b12, b21 + b22]


def _mc(c11, c12, c21, c22):
    return [c11 + c22, c21 - c22, c12 + c22, c11 + c21, c12 - c11, c22, c11]


def _post(m):
    return m[0] + m[3] - m[4] + m[6], m[2] + m[4], m[1] + m[3], m[0] - m[1] + m[2] + m[5]


def _post_l(m):
    return m[0] + m[2] + m[4] - m[5], m[4] + m[6], m[1] + m[5], m[0] + m[1] + m[3] - m[6]


def _post_r(m):
    return m[0] + m[1] - m[3] + m[5], m[2] + m[5], m[3] + m[6], m[0] - m[2] + m[4] + m[6]


_REM1 = (0, 1, 2, 5)
_REM2 = (0, 1, 3, 6)
_ROWS = [(r, r, 256 + r) for r in range(0, 256, 16)] + [(256 + r, 512 + r, 544 + r) for r in (0, 16)]


def _radix4(x, sign):
    (ar, ai), (br, bi), (cr, ci), (dr, di) = x
    t0r, t0i, t1r, t1i = ar + cr, ai + ci, ar - cr, ai - ci
    t2r, t2i, t3r, t3i = br + dr, bi + di, br - dr, bi - di
    p = (t1r + t3i, t1i - t3r)
    m = (t1r - t3i, t1i + t3r)
    y1, y3 = (p, m) if sign < 0 else (m, p)
    return [(t0r + t2r, t0i + t2i), y1, (t0r - t2r, t0i - t2i), y3]


def _twiddle(z, e, sign):
    r, i = z
    if e == 0:
        return z
    if e == 4:
        return (i, -r) if sign < 0 else (-i, r)
    c = float(np.cos(2 * np.pi * e / 16))
    s = float(sign * np.sin(2 * np.pi * e / 16))
    if e in (2, 6):
        return ((r - i) * c, (r + i) * c) if c * s > 0 else ((r + i) * c, (i - r) * c)
    return (r * c - i * s, r * s + i * c)


def _fft16(x, sign):
    a = [_radix4([x[b], x[4 + b], x[8 + b], x[12 + b]], sign) for b in range(4)]
    out = [None] * 16
    for c in range(4):
        y = _radix4([_twiddle(a[b][c], b * c, sign) for b in range(4)], sign)
        for d in range(4):
            out[c + 4 * d] = y[d]
    return out


def _radix6(n):
    e = [n[j] + n[j + 3] for j in range(3)]
    o = [n[j] - n[j + 3] for j in range(3)]
    es, od = e[1] + e[2], o[1] - o[2]
    return [e[0] + es, o[0] - od, o[0] + 0.5 * od, o[1] + o[2], e[0] - 0.5 * es, e[1] - e[2]]


def _radix6_adj(t):
    t0, t3, p1, q1, p2, q2 = t
    es, od = t0 - 0.5 * p2, 0.5 * p1 - t3
    e = [t0 + p2, es + q2, es - q2]
    o = [t3 + p1, q1 + od, q1 - od]
    return [e[j] + o[j] for j in range(3)] + [e[j] - o[j] for j in range(3)]


def _barrel(v, cls):
    w = [v[(-m) % 16] for m in range(16)]
    for b in range(4):
        m = (cls & (1 << b)) != 0
        w = [jnp.where(m, w[(i - (1 << b)) % 16], w[i]) for i in range(16)]
    return w


def _total(vs):
    acc = vs[0]
    for v in vs[1:]:
        acc = acc + v
    return acc[:8] + acc[8:]


def _mean(acc):
    return jnp.sum(acc, axis=0, keepdims=True) * (1.0 / D)


def _sums(n, count, width, body):
    def step(i, acc):
        return tuple(a + _total(v) for a, v in zip(acc, body(i)))
    acc = jax.lax.fori_loop(0, n, step, (jnp.zeros((8, width), F32),) * count)
    return [_mean(a) for a in acc]


def _loop(n, body):
    def step(i, c):
        body(i)
        return c
    jax.lax.fori_loop(0, n, step, 0)


def _ds(start, n):
    return pl.ds(start if isinstance(start, int) else pl.multiple_of(start, n), n)


def _paced(dots, costs, pieces, fence, frac=0.85):
    done, cum, span = 0, 0, sum(costs) * frac
    for t, w in zip(dots, costs):
        v = t()
        nr = v.shape[0] // 16
        while done < len(pieces) and done * span < (cum + w) * len(pieces):
            r = min(nr - 1, int((done * span / len(pieces) - cum) / w * nr))
            fence(v[r * 16:r * 16 + 16, :128])
            pieces[done]()
            done += 1
        cum += w


def _kernel(x_hbm, go_hbm, wr_hbm, wi_hbm, cm_hbm, g_hbm, wg_hbm, wu_hbm, wd_hbm,
            out_hbm, dx_hbm, dwr_hbm, dwi_hbm, dwg_hbm, dwu_hbm, dwd_hbm,
            xT, goT, wbw, wl, cm, g, wp, dwp, tb, z, zb, xs, h, dh, st, ob,
            lnT, mgT, ln, mg, rem, stage, turn, hacc, dacc, wacc, m, dm, rw, wst, gst,
            zs, sems, xsem, wsem, gsem):
    w_hbm = (wg_hbm, wu_hbm, wd_hbm)
    dw_hbm = (dwg_hbm, dwu_hbm, dwd_hbm)
    wb = wbw.bitcast(BF)

    def x_copy(c):
        return pltpu.make_async_copy(x_hbm.at[:, _ds(c * XC, XC)], xT.at[:, _ds(c * XC, XC)],
                                     xsem.at[c])

    def gg_copies(c):
        return [pltpu.make_async_copy(g_hbm.at[pl.ds(4 * c, 4)], g.at[pl.ds(4 * c, 4)],
                                      xsem.at[4 + c])] + [
            pltpu.make_async_copy(go_hbm.at[:, _ds(i * SH + c * 256, 256)],
                                  goT.at[:D, _ds(i * SH + c * 256, 256)], xsem.at[8 + 4 * i + c])
            for i in range(2)]

    def cm_copy(i):
        return pltpu.make_async_copy(cm_hbm.at[i], cm.at[i], sems.at[i])

    def tile_copy(name, t):
        cols = _ds(t * 128, 128)
        if name == "out":
            return pltpu.make_async_copy(ob.at[t], out_hbm.at[:, cols], sems.at[8])
        ref, a, load = {"wr": (wr_hbm, 0, 1), "wi": (wi_hbm, 1, 1),
                        "dwr": (dwr_hbm, 0, 0), "dwi": (dwi_hbm, 1, 0)}[name]
        ends = (ref.at[:288, cols], wb.at[16 * a + t, :288])
        return pltpu.make_async_copy(*(ends if load else ends[::-1]), sems.at[9])

    def all_tiles(name):
        if name == "out":
            return pltpu.make_async_copy(ob, ob, sems.at[8])
        return pltpu.make_async_copy(wb.at[:, :288], wb.at[:, :288], sems.at[9])

    def last_row_copies(load):
        ends = [(ref.at[288:], wl.at[a, 16:])
                for a, ref in enumerate((wr_hbm, wi_hbm) if load else (dwr_hbm, dwi_hbm))]
        return [pltpu.make_async_copy(*(e if load else e[::-1]), sems.at[2 + a])
                for a, e in enumerate(ends)]

    def w_copies(j):
        return [pltpu.make_async_copy(w_hbm[i].at[:, _ds(j * TF, TF)], wst.at[(j % 2) * 3 + i],
                                      wsem.at[(j % 2) * 3 + i]) for i in range(3)]

    def dw_copies(j):
        return [pltpu.make_async_copy(gst.at[(j % 2) * 3 + i], dw_hbm[i].at[:, _ds(j * TF, TF)],
                                      gsem.at[(j % 2) * 3 + i]) for i in range(3)]

    def start(cs):
        for c in cs:
            c.start()

    def wait(cs):
        for c in cs:
            c.wait()

    def fence(ref, index):
        def put(v):
            if ref.ndim == 2:
                ref[_ds(zs[0] + index, 16), :128] = v.astype(ref.dtype)
            else:
                ref[zs[0] + index, :16, :128] = v.astype(ref.dtype)
        return put

    def wcomb_pieces(b, q):
        def pair(i, c, ra, rb, rd):
            lo, hi = slice(c, c + 128), slice(FH + c, FH + c + 128)
            w = [wst[b * 3 + i, r, cs].astype(F32) for r in (ra, rb) for cs in (lo, hi)]
            vs = _rc(*w) if i < 2 else _rc(w[0], w[2], w[1], w[3])
            for k in range(7):
                rw[b * 7 + k, rd, i * FH + c:i * FH + c + 128] = _wd(vs[k])

        def tail(i, c):
            rs = _ds(512 + q * 16, 16)
            top, bot = _ds(144 + q * 8, 8), _ds(176 + q * 8, 8)
            cs = slice(i * FH + c, i * FH + c + 128)
            u, v = wst[b * 3 + i, rs, c:c + 128], wst[b * 3 + i, rs, FH + c:FH + c + 128]
            rw[b * 7, top, cs] = _wd(u)
            rw[b * 7 + 1, bot, cs] = _wd(u)
            if i < 2:
                t = u.astype(F32) + v.astype(F32)
                rw[b * 7 + 2, top, cs] = _wd(v)
                rw[b * 7 + 5, top, cs] = _wd(-t)
                rw[b * 7 + 5, bot, cs] = _wd(t)
            else:
                t = _wd(v.astype(F32) - u.astype(F32))
                rw[b * 7 + 3, top, cs] = t
                rw[b * 7 + 3, bot, cs] = t
                rw[b * 7 + 6, top, cs] = _wd(v)
        ps = []
        for i in range(3):
            for c in range(0, FH, 128):
                for r in range(0, 64, 16):
                    ps.append(lambda i=i, c=c, r=r: pair(
                        i, c, _ds(q * 64 + r, 16), _ds(256 + q * 64 + r, 16), _ds(q * 32 + r // 2, 8)))
                hq = q % 2
                ps.append(lambda i=i, c=c: (pair(i, c, _ds(512 + hq * 16, 16), _ds(544 + hq * 16, 16),
                                                 _ds(128 + hq * 8, 8)), tail(i, c)))
        return ps

    def wpost_pieces(b, q):
        def piece(i, c, rs, ra, rb):
            lo, hi = slice(c, c + 128), slice(FH + c, FH + c + 128)
            v = _post_r([wacc[b * 7 + k, rs, i * FH + c:i * FH + c + 128] for k in range(7)])
            if i == 2:
                v = (v[0], v[2], v[1], v[3])
            for t, (r, cs) in zip(v, ((ra, lo), (ra, hi), (rb, lo), (rb, hi))):
                gst[b * 3 + i, r, cs] = t.astype(BF)
        ps = []
        for i in range(3):
            for c in range(0, FH, 128):
                for r in range(0, 64, 16):
                    ra = _ds(q * 64 + r, 16)
                    ps.append(lambda i=i, c=c, ra=ra, r=r: piece(i, c, ra, ra, _ds(256 + q * 64 + r, 16)))
                hq = (q % 2) * 16
                ps.append(lambda i=i, c=c: piece(i, c, _ds(256 + hq, 16), _ds(512 + hq, 16),
                                                 _ds(544 + hq, 16)))
        return ps

    def transpose_pieces(i, src, dst, c):
        def full(k):
            dst[k, _ds(c * 64, 64)] = pltpu.bitcast(_bf(src(k, 128)).T, U32)

        def tail():
            rem[i, _ds(c * 64, 64)] = pltpu.bitcast(_bf(src(7, 64)).T, U32)
        return [lambda k=k: full(k) for k in range(7)] + [tail]

    def put_combos(dsts, comb, rd, a, b):
        vs = [(k, rd // 2, v) for k, v in enumerate(comb(a[0], a[1], b[0], b[1]))]
        if rd >= 256:
            vs += [(7, 16 * i + (rd - 256) // 2, v) for i, v in enumerate((a[0], a[1], b[0], b[1]))]
        for k, r, v in vs:
            w = _wd(v)
            for dst in dsts:
                ref, idx = dst(k, slice(r, r + 8))
                ref[idx] = w

    def go_pieces(c):
        def piece(rd, ra, rb):
            a, b = [[goT[r:r + 16, _ds(s + c * 128, 128)].astype(F32) for r in (ra, rb)]
                    for s in (0, SH)]
            put_combos([lambda k, r: (mgT, (k, r, _ds(c * 128, 128)))], _mc, rd, a, b)
        return [lambda r=r: piece(*r) for r in _ROWS] + [
            lambda: [t() for t in transpose_pieces(
                1, lambda k, n: mgT[k, :n, _ds(c * 128, 128)], mg, c)]]

    def out_pieces(c):
        def piece(rd, ra, rb):
            f = _post([hacc[k, rd:rd + 16, _ds(c * 128, 128)] for k in range(7)])
            for v, (i, r) in zip(f, ((0, ra), (0, rb), (1, ra), (1, rb))):
                ob[8 * i + c, r:r + 16] = (h[r:r + 16, _ds(i * SH + c * 128, 128)] + v).astype(BF)
        return [lambda r=r: piece(*r) for r in _ROWS]

    def rows6(i):
        return [_ds(96 * j + 16 * i, 16) for j in range(6)]

    def split_rows(i):
        return (_ds(16 * i, 16), _ds(16 * i + jnp.where(i < 16, 0, 256), 16),
                _ds(16 * i + jnp.where(i < 16, 256, 288), 16))

    def rows(ref, i, cols):
        return [ref[r, cols].astype(F32) for r in rows6(i)]

    def put_rows(ref, i, cols, vs):
        for r, v in zip(rows6(i), vs):
            ref[r, cols] = v

    def put_radix6(n, i, cols):
        for j, t in enumerate(_radix6(n)):
            tb[_ds(48 * j + 8 * i, 8), cols] = _wd(t)

    def ln_bwd_stats(i, cols, m1, m2):
        mu, r = st[i:i + 1, cols], st[i + 1:i + 2, cols]
        c1 = (m2 - mu * m1) * (r * r * r)
        st[4:5, cols] = r * m1 - c1 * mu
        st[5:6, cols] = c1

    def ln_bwd(i, cols, res, dn, x):
        r, c0, c1 = st[i + 1:i + 2, cols], st[4:5, cols], st[5:6, cols]
        return [a + (r * d - (c0 + c1 * v)) for a, d, v in zip(res, dn, x)]

    def fwd_pre():
        start([x_copy(c) for c in range(S // XC)] + [cm_copy(0)])
        zs[0] = 0
        wbw[:, 144:] = jnp.zeros((32, 24, 128), U32)
        rw[:, 144:] = jnp.zeros((14, 64, 3 * FH), U32)

        def stats(c):
            x_copy(c).wait()
            start([tile_copy(n, 4 * c + t) for n in ("wr", "wi") for t in range(4)])

            cols = _ds(c * XC, XC)
            mu, = _sums(6, 1, XC, lambda i: [rows(xT, i, cols)])

            def var(i):
                xc = [v - mu for v in rows(xT, i, cols)]
                put_radix6(xc, i, cols)
                return [[v * v for v in xc]]
            st[0:1, cols] = mu
            st[1:2, cols] = jax.lax.rsqrt(_sums(6, 1, XC, var)[0] + EPS)
        _loop(S // XC, stats)
        start(last_row_copies(True))
        cm_copy(0).wait()

    def spectral(ph):
        def d_units(c):
            for gi in (2, 3, 0, 1):
                w = 256 if gi >= 2 else 512
                for q in range(0, 1024, w):
                    yield (gi,) + _GRP[gi] + (c * 1024 + q, w)

        def dfwd(c):
            def t(gi, o, n, t0, k, c0, w):
                cols = _ds(c0, w)
                v = _dot(_bf(cm[0, gi, :n, :k]), _bf(tb[t0 // 2:(t0 + k) // 2, cols]))
                v = v * jnp.where(ph == 0, st[1:2, cols], 1.0)
                z[o:o + n, cols] = v[:n]
                z[FP + o:FP + o + n, cols] = v[n:]
                return v
            us = list(d_units(c))
            _paced([lambda u=u: t(*u) for u in us], [u[2] for u in us],
                   sum([out_pieces(4 * c + i) for i in range(4)], []), fence(hacc, 7))
        _loop(2, dfwd)

        cls = jax.lax.broadcasted_iota(jnp.int32, (8, 128), 1) & 15

        def pair_rows(i):
            w0 = 24 * i
            for q in (1, 2):
                w0 = jnp.where(i >= _PAIR[q][0] // 8, q + 24 * (i - _PAIR[q][0] // 8), w0)
            return pl.ds(w0, 8, stride=3)

        def load_z(r):
            return [(z[_ds(r, 8), t * 128:(t + 1) * 128],
                     z[_ds(FP + r, 8), t * 128:(t + 1) * 128]) for t in range(16)]

        def bfly(i):
            a = _fft16(load_z(i * 16), -1)
            z[_ds(zs[0] + 2 * FP, 8), :128] = a[15][1]
            b = _fft16(load_z(i * 16 + 8), -1)
            for k in range(16):
                zb[k, _ds(i * 8, 8), :128] = _stack(a[k][0], b[k][0])
                zb[k, _ds(i * 8, 8), 128:] = _stack(a[k][1], b[k][1])

        def roll_in(i):
            for t in range(32):
                v = wbw[t, pair_rows(i)]
                turn[t] = pltpu.roll(v, t % 16, 1) if t % 16 else v

        def bfly_perm(i):
            for a in range(2):
                v = _barrel([turn[16 * a + t] for t in range(16)], cls)
                for k in range(16):
                    wp[2 * k + a, _ds(i * 8, 8)] = v[k]
            roll_in(jnp.minimum(i + 1, FP // 16 - 1))
            bfly(i)

        @pl.when(ph == 0)
        def _():
            start(gg_copies(0) + gg_copies(1))
            wait([all_tiles("w")] + last_row_copies(True))
            top = jax.lax.broadcasted_iota(jnp.int32, (8, 128), 0) == 0
            for t in range(32):
                v = wl[t // 16, 16:, t % 16 * 128:(t % 16 + 1) * 128].astype(F32)
                wbw[t, 144:152] = _both(jnp.where(top, v, 0.0), jnp.zeros((8, 128), F32))
            roll_in(0)
            _loop(FP // 16, bfly_perm)

        @pl.when(ph == 1)
        def _():

            def bfly_out(i):
                pl.when(i < 16)(lambda: tile_copy("out", i).start())
                bfly(i)
            _loop(FP // 16, bfly_out)

        row = jax.lax.broadcasted_iota(jnp.int32, (64, 128), 0)
        cf = jnp.concatenate([jnp.where((row == 0) | (row == 48), 1.0 / (S * D), 2.0 / (S * D)),
                              jnp.full((FP - 64, 128), 2.0 / (S * D), F32)], axis=0)
        sg = jnp.where(ph == 0, 1.0, -1.0)
        z8 = jnp.zeros((8, 128), F32)

        def unpair(w):
            parts = {r: _half(w[_PAIR[r // 2][0]:_PAIR[r // 2][0] + min(n, 56)], r % 2)
                     for r, (_, n) in _CLS.items()}
            return jnp.concatenate([parts[0], z8] + [parts[r] for r in (3, 1, 5, 2, 4)], axis=0)

        def pair(v):
            c = {r: v[o:o + min(n, 56)] for r, (o, n) in _CLS.items()}
            c[1] = jnp.concatenate([c[1], z8], axis=0)
            return jnp.concatenate([_both(c[2 * q], c[2 * q + 1]) for q in range(3)], axis=0)

        def mix(i):
            @pl.when(ph == 0)
            def _():
                pl.when(i < 2)(lambda: start(gg_copies(i + 2)))
                pl.when(i == 1)(lambda: start(w_copies(0) + [cm_copy(1)]))
                pl.when(i == 3)(lambda: start(w_copies(1)))
                wait(gg_copies(i))
            ys = {}

            def fwd(kk):
                k = i * 4 + kk
                v = _dot(_bf(zb[k]), _bf(g[k]))
                vr, vi = v[:, :128], v[:, 128:]
                gr, gi = vr * cf, vi * cf
                xr, xi = xs[2 * k], xs[2 * k + 1]
                wr, wi = unpair(wp[2 * k]), unpair(wp[2 * k + 1]) * sg
                dwp[2 * k] = pair(gr * xr + gi * xi)
                dwp[2 * k + 1] = pair(gi * xr - gr * xi)
                xs[2 * k] = vr
                xs[2 * k + 1] = vi
                ys[kk] = jnp.concatenate([(gr * wr - gi * wi).astype(BF),
                                          (gr * wi + gi * wr).astype(BF)], axis=1)
                return v

            def inv(kk):
                k = i * 4 + kk
                v = _dot_nt(ys[kk], _bf(g[k]))
                z[:FP, _ds(k * 128, 128)] = v[:, :128]
                z[FP:2 * FP, _ds(k * 128, 128)] = v[:, 128:]
                return v
            for kk in range(4):
                fwd(kk)
            _paced([lambda kk=kk: inv(kk) for kk in range(4)], (1, 1, 1, 1),
                   go_pieces(2 * i) + go_pieces(2 * i + 1), fence(goT, D), 0.7)
        _loop(4, mix)

        def ibfly(i):
            y = _fft16(load_z(i * 8), 1)
            for t in range(16):
                tb[_ds(i * 8, 8), t * 128:(t + 1) * 128] = _stack(*y[t])

        def roll_out(i):
            for t in range(32):
                wbw[t, pair_rows(i)] = pltpu.roll(turn[t], 128 - t % 16, 1) if t % 16 else turn[t]

        def ibfly_unperm(i):
            roll_out(jnp.maximum(i - 1, 0))
            for a in range(2):
                v = _barrel([dwp[2 * k + a, _ds(i * 8, 8)] for k in range(16)], cls)
                for t in range(16):
                    turn[16 * a + t] = v[t]
            ibfly(2 * i)
            z[_ds(zs[0] + 2 * FP, 8), :128] = pltpu.bitcast(tb[_ds(i * 16, 8), 1920:], F32)
            ibfly(2 * i + 1)

        @pl.when(ph == 0)
        def _():
            _loop(FP // 8, ibfly)
            wait(w_copies(0) + [cm_copy(1)])

        @pl.when(ph == 1)
        def _():
            _loop(FP // 16, ibfly_unperm)
            roll_out(FP // 16 - 1)
            for t in range(32):
                wl[t // 16, 16:, t % 16 * 128:(t % 16 + 1) * 128] = (
                    _half(wbw[t, 144:152], 0)[:1].astype(BF))
            start(last_row_copies(False))

        def dinv(c):
            pl.when(ph == 1)(lambda: start(
                [tile_copy(n, 8 * c + t) for n in ("dwr", "dwi") for t in range(8)]))

            def t(gi, o, n, t0, k, c0, w):
                v = _dot(_bf(cm[1, gi, :k // 2, :2 * n]), _bf(tb[o:o + n, _ds(c0, w)]))
                z[t0:t0 + k, _ds(c0, w)] = v
                return v
            us = list(d_units(c))
            _paced([lambda u=u: t(*u) for u in us], [u[4] for u in us],
                   wcomb_pieces(0, 2 * c) + wcomb_pieces(0, 2 * c + 1), fence(wst, 6))
        _loop(2, dinv)

    def fwd_post():
        def stats(c):
            cols = _ds(c * 512, 512)

            def resid(i):
                hv = [a + b for a, b in zip(rows(xT, i, cols), _radix6_adj(rows(z, i, cols)))]
                put_rows(h, i, cols, hv)
                return [hv]
            mu, = _sums(6, 1, 512, resid)
            var, = _sums(6, 1, 512, lambda i: [[(v - mu) * (v - mu) for v in rows(h, i, cols)]])
            st[2:3, cols] = mu
            st[3:4, cols] = jax.lax.rsqrt(var + EPS)
        _loop(S // 512, stats)

        def norm(c):
            for t in range(2):
                for p in transpose_pieces(0, lambda k, n: stage[1 - t, k, :n], ln, (2 * c + t + 7) % 8):
                    p()
                cols = [_ds(s + c * 256 + t * 128, 128) for s in (0, SH)]
                for rd, ra, rb in _ROWS:
                    put_combos([lambda k, r: (lnT, (k, r, cols[0])), lambda k, r: (stage, (t, k, r))],
                               _lc, rd, *[[(h[r:r + 16, q] - st[2:3, q]) * st[3:4, q] for r in (ra, rb)]
                                          for q in cols])
        _loop(SH // 256, norm)
        for p in transpose_pieces(0, lambda k, n: stage[1, k, :n], ln, 7):
            p()

    def ffn_tile(j):
        pl.when(j + 1 < NF)(lambda: wait(w_copies(j + 1)))
        pl.when(j + 2 < NF)(lambda: start(w_copies(j + 2)))
        pl.when(j >= 2)(lambda: start(dw_copies(j - 2)))
        pl.when(j >= 3)(lambda: wait(dw_copies(j - 3)))
        _loop(NC, lambda c: ffn_iter(j, c))

    def ffn_iter(j, c):
        b = j % 2
        s0 = c * SC
        parts = ((slice(0, TF), ln, lnT, dacc, _REM1), (slice(TF, 3 * FH), mg, mgT, hacc, _REM2))

        def p_dots(o):
            rs = _ds((s0 + o) // 2, SUB // 2)

            def t(i, k):
                cs, lhs, _, _, has_rem = parts[i]
                a, w = lhs[k, rs], rw[b * 7 + k, :128, cs]
                if k in has_rem:
                    a = jnp.concatenate([a, rem[i, rs]], axis=1)
                    w = jnp.concatenate([w, rw[b * 7 + k, 144:, cs]], axis=0)
                v = _dot(_bf(a), _bf(w))
                m[k, o:o + SUB, cs] = v
                return v
            return [lambda i=i, k=k: t(i, k) for i in range(2) for k in range(7)]

        def r_dots(o):
            rs = _ds(s0 + o, SUB)

            def t(i, k):
                cs, _, _, acc, _ = parts[i]
                v = (jnp.where(j == 0, 0.0, acc[k, :, rs])
                     + _dot_nt(_bf(rw[b * 7 + k, :144, cs]), _bf(dm[k, o // 2:(o + SUB) // 2, cs])))
                acc[k, :, rs] = v
                return v
            return [lambda i=i, k=k: t(i, k) for i in range(2) for k in range(7)]

        def q_dots():
            def t(i, k):
                cs, _, lhs, _, _ = parts[i]
                v = (jnp.where(c == 0, 0.0, wacc[b * 7 + k, :, cs])
                     + _dot(_bf(lhs[k, :, _ds(s0, SC)]), _bf(dm[k, :, cs])))
                wacc[b * 7 + k, :, cs] = v
                return v
            return [lambda i=i, k=k: t(i, k) for i in range(2) for k in range(7)]

        def ew_pieces(o):
            def piece(r, c0):
                rs = slice(r, r + 16)
                cs = [slice(i * FH + c0, i * FH + c0 + 128) for i in range(3)]
                a = _post([m[k, rs, cs[0]] for k in range(7)])
                u = _post([m[k, rs, cs[1]] for k in range(7)])
                dp = _post_l([m[k, rs, cs[2]] for k in range(7)])
                da, du, p = [], [], []
                for ai, ui, di in zip(a, u, dp):
                    s = 0.5 * jnp.tanh(0.5 * ai) + 0.5
                    gl = ai * s
                    p.append(gl * ui)
                    du.append(di * gl)
                    da.append((di * ui) * (s + gl * (1.0 - s)))
                for cc, vs in zip(cs, (_mc(*da), _mc(*du), _lc(*p))):
                    for k in range(7):
                        dm[k, r // 2:r // 2 + 8, cc] = _wd(vs[k])
            return [lambda r=r, c0=c0: piece(r, c0)
                    for r in range(o, o + SUB, 16) for c0 in range(0, FH, 128)]

        costs = [2] * 7 + [1] * 7
        _paced(p_dots(0), costs, wpost_pieces(1 - b, c), fence(wacc, 14))
        _paced(p_dots(SUB), costs, ew_pieces(0), fence(m, 7))
        _paced(r_dots(0), costs, ew_pieces(SUB), fence(m, 7))
        _paced(r_dots(SUB), costs, [], None)
        _paced(q_dots(), costs, wcomb_pieces(1 - b, c), fence(wst, 6))

    def bwd_pre():
        start(dw_copies(NF - 2))

        def sums(c):
            cols = [_ds(s + c * 256, 256) for s in (0, SH)]

            def part(i):
                rd, ra, rb = split_rows(i)
                v = _post_l([dacc[k, rd, cols[0]] for k in range(7)])
                w = []
                for t, (q, r) in zip(v, ((0, ra), (0, rb), (1, ra), (1, rb))):
                    z[r, cols[q]] = t
                    w.append(t * h[r, cols[q]])
                return [v[:2], w[:2], v[2:], w[2:]]
            ms = _sums(18, 4, 256, part)
            ln_bwd_stats(2, cols[0], ms[0], ms[1])
            ln_bwd_stats(2, cols[1], ms[2], ms[3])
        _loop(SH // 256, sums)

        def apply(it):
            i, cols = it % 6, _ds(it // 6 * 512, 512)
            dv = ln_bwd(2, cols, rows(goT, i, cols), rows(z, i, cols), rows(h, i, cols))
            put_rows(dh, i, cols, dv)
            put_radix6(dv, i, cols)
        _loop(6 * S // 512, apply)
        wait(dw_copies(NF - 3))

        def post(q):
            for p in wpost_pieces((NF - 1) % 2, q):
                p()
        _loop(NC, post)
        start(dw_copies(NF - 1))

    def bwd_post():
        wait([all_tiles("out")] + last_row_copies(False) + dw_copies(NF - 2) + dw_copies(NF - 1))

        def chunk(c):
            cols = _ds(c * 512, 512)

            def part(i):
                t = rows(z, i, cols)
                dn = _radix6_adj(t)
                put_rows(h, i, cols, dn)
                return [t[:1], [d * v for d, v in zip(dn, rows(xT, i, cols))]]
            m0, m2 = _sums(6, 2, 512, part)
            ln_bwd_stats(0, cols, 6.0 * m0, m2)

            def apply(i):
                rs = [_ds(96 * i + 16 * j, 16) for j in range(6)]
                dv = ln_bwd(0, cols, *[[ref[r, cols].astype(F32) for r in rs] for ref in (dh, h, xT)])
                for r, v in zip(rs, dv):
                    goT[r, cols] = v.astype(BF)
                pltpu.make_async_copy(goT.at[_ds(96 * i, 96), cols], dx_hbm.at[_ds(96 * i, 96), cols],
                                      sems.at[4]).start()
            _loop(6, apply)
        _loop(S // 512, chunk)
        wait([all_tiles("w")] + [pltpu.make_async_copy(goT.at[:D], dx_hbm, sems.at[4])])

    def phase(ph):
        pl.when(ph == 0)(fwd_pre)
        pl.when(ph == 1)(bwd_pre)
        spectral(ph)

        @pl.when(ph == 0)
        def _():
            fwd_post()
            _loop(NF, ffn_tile)
        pl.when(ph == 1)(bwd_post)
    _loop(2, phase)


@jax.jit
def pallas_sequential_preLN__spectral_gfnet__swiglu_ffn__prompt_kernel(
    A_x, A_w_r, A_w_i, B_x, B_w_gate, B_w_up, B_w_down, grad_out,
):
    del B_x
    anyspec = pl.BlockSpec(memory_space=pl.ANY)
    sds = jax.ShapeDtypeStruct
    V = pltpu.VMEM
    dma = pltpu.SemaphoreType.DMA
    outs = pl.pallas_call(
        _kernel,
        in_specs=[anyspec] * 9,
        out_specs=[anyspec] * 7,
        out_shape=[sds((D, S), BF), sds((D, S), BF), sds((DF, S), BF), sds((DF, S), BF),
                   sds((D, F), BF), sds((D, F), BF), sds((D, F), BF)],
        scratch_shapes=[
            V((D, S), BF),
            V((D + 16, S), BF),
            V((32, 168, 128), U32),
            V((2, 17, S), BF),
            V((2, 4, 96, 256), U32),
            V((16, 128, 256), U32),
            V((32, FP // 2, 128), U32),
            V((32, FP // 2, 128), U32),
            V((FP, S), U32),
            V((2 * FP + 8, S), F32),
            V((16, FP // 2, 256), U32),
            V((32, FP, 128), F32),
            V((D, S), F32),
            V((D, S), F32),
            V((8, S), F32),
            V((16, D, 128), BF),
            V((8, 144, SH), U32),
            V((8, 144, SH), U32),
            V((7, SH // 2, 256), U32),
            V((7, SH // 2, 256), U32),
            V((2, SH // 2, 128), U32),
            V((2, 8, 144, 128), U32),
            V((32, 8, 128), U32),
            V((8, 288, SH), F32),
            V((7, 288, SH), F32),
            V((15, 288, 3 * FH), F32),
            V((8, SC, 3 * FH), F32),
            V((7, SC // 2, 3 * FH), U32),
            V((14, 208, 3 * FH), U32),
            V((7, D, TF), BF),
            V((6, D, TF), BF),
            pltpu.SMEM((1,), jnp.int32),
            dma((10,)), dma((16,)), dma((6,)), dma((6,)),
        ],
        compiler_params=pltpu.CompilerParams(vmem_limit_bytes=124 * 1024 * 1024,
                                             disable_bounds_checks=True),
        name="fused_gfnet_swiglu",
    )(A_x[0].T, grad_out[0].T, A_w_r.T, A_w_i.T, _CM, _G, B_w_gate, B_w_up, B_w_down.T)
    o, dx, dwr, dwi, dwg, dwu, dwd = outs
    return (o.T[None], dx.T[None], dwr.T, dwi.T, dwg, dwu, dwd.T)
```
